```python
import os as _os
_os.environ.setdefault("JAX_PLATFORMS", "cpu")
import jax
import jax.numpy as jnp

def _softmax(x, axis=-1):
    return jax.nn.softmax(x, axis=axis)
def _gelu(x):
    return jax.nn.gelu(x, approximate=True)
def _silu(x):
    return jax.nn.silu(x)
def _sigmoid(x):
    return jax.nn.sigmoid(x)
def _layernorm(x, axis=-1, eps=1e-5):
    m = jnp.mean(x, axis=axis, keepdims=True)
    v = jnp.var(x, axis=axis, keepdims=True)
    return (x - m) / jnp.sqrt(v + eps)
def _scatter_add(tgt, idx, src, axis=0):
    return tgt.at[idx].add(src)
def _segment_sum(src, seg, n):
    return jax.ops.segment_sum(src, seg, n)
class _Rng:
    def __init__(self, key):
        self._k = key
    def _next(self):
        self._k, sub = jax.random.split(self._k)
        return sub
    def normal(self, shape):
        return jax.random.normal(self._next(), shape, dtype=jnp.bfloat16)
    def randint(self, lo, hi, shape):
        return jax.random.randint(self._next(), shape, lo, hi, dtype=jnp.int32)
    def uniform(self, shape, lo=0.0, hi=1.0):
        return jax.random.uniform(self._next(), shape, jnp.bfloat16, lo, hi)
    def permutation(self, n):
        return jax.random.permutation(self._next(), n)


kernel_name = 'gated_mix__spectral_gfnet__dense_activation_silu__prompt'

def setup_inputs():
    _rng = _Rng(jax.random.key(int.from_bytes(__import__("os").urandom(4), "little")))
    _w = (lambda a: (lambda t: t.astype(jnp.bfloat16) if jnp.issubdtype(t.dtype, jnp.floating) else t)(jnp.asarray(a)))
    def _A_setup():
        B, S, D = 1, 2048, 512
        Df = D // 2 + 1
        return {
            "x": _w((lambda *s: _rng.normal(s) * 0.05)(B, S, D)),
            "w_r": _w((lambda *s: _rng.normal(s) * 0.05)(S, Df) * 0.02),
            "w_i": _w((lambda *s: _rng.normal(s) * 0.05)(S, Df) * 0.02),
        }
    _A_in = _A_setup()

    def _B_setup():
        B, S, D, F = 1, 2048, 512, 1376
        return {
            "x": _w((lambda *s: _rng.normal(s) * 0.05)(B, S, D)),
            "w1": _w((lambda *s: _rng.normal(s) * 0.05)(D, F) * (D ** -0.5)),
            "w2": _w((lambda *s: _rng.normal(s) * 0.05)(F, D) * (F ** -0.5)),
        }
    _B_in = _B_setup()

    return {
        "A_x": _A_in["x"],
        "A_w_r": _A_in["w_r"],
        "A_w_i": _A_in["w_i"],
        "B_x": _B_in["x"],
        "B_w1": _B_in["w1"],
        "B_w2": _B_in["w2"],
        "gate_w": _w((lambda *s: _rng.normal(s) * 0.05)(512) * 16.0),
    }

def reference(A_x, A_w_r, A_w_i, B_x, B_w1, B_w2, gate_w):
    def _A_ref(x, w_r, w_i):
        B, S, D = x.shape
        X = (lambda x, axes=(-2,-1): jnp.fft.rfft2(x.astype(jnp.float32), axes=axes))(x, axes=(-2, -1))
        W = w_r + 1j * w_i
        X = X * W
        y = (lambda x, s, axes=(-2,-1): jnp.fft.irfft2(x, s=s, axes=axes).astype(jnp.bfloat16))(X, (S, D), axes=(-2, -1))
        return y

    def _B_ref(x, w1, w2):
        h = jnp.einsum("bsd,df->bsf", x, w1)
        h = _silu(h)
        out = jnp.einsum("bsf,fd->bsd", h, w2)
        return out

    x = A_x
    g = _sigmoid((x * gate_w).sum(-1, keepdims=True))
    a = _A_ref(x, A_w_r, A_w_i)
    b = _B_ref(x, B_w1, B_w2)
    return g * a + (1 - g) * b
```

```python
import numpy as np
import jax
import jax.numpy as jnp
import jax.experimental.pallas as pl
import jax.experimental.pallas.tpu as pltpu

S, D, F = 2048, 512, 1376
BF, F32 = jnp.bfloat16, jnp.float32


def _gen(gidx, fef, foo, fs, gs, c1, f64, tw):
    def io(shape, d):
        return jax.lax.broadcasted_iota(jnp.int32, shape, d)

    def cs(j):
        return jnp.cos((j & 2047).astype(F32) * np.float32(2 * np.pi / 2048))
    Q = 512
    r, l = io((128, 128), 0), io((128, 128), 1)
    r8 = r[:8]

    def ex(k, ph=0, n=16):
        k, ph = k[:8], (ph + 0 * l)[:8]
        c0, s0 = cs(r8 * k + ph), cs(r8 * k + ph + Q)
        o = []
        for h in range(0, n, 8):
            c1_, s1 = cs(8 * (r8 + h) * k), cs(8 * (r8 + h) * k + Q)
            o += [(c0 * c1_[i:i + 1] - s0 * s1[i:i + 1], c0 * s1[i:i + 1] + s0 * c1_[i:i + 1])
                  for i in range(min(8, n))]
        return jnp.concatenate([a for a, _ in o], 0), jnp.concatenate([b for _, b in o], 0)
    q, m = l >> 5, l & 31
    sw = ((q & 1) << 1) | (q >> 1)
    gidx[0] = (4 * m + sw)[:8]
    gidx[1] = (4 * m + (sw ^ 1))[:8]
    ke = 4 * m + 128 * (q >> 1)
    kf = jnp.where(q & 1 == 1, ke, 4 * m + 128 - 128 * (q >> 1)) + 2
    fe = ex(4 * ke, Q * (q & 1))[0]
    fe = jnp.where(l == 32, (1 - 2 * (r & 1)).astype(F32), fe)
    ff = ex(4 * kf, Q * (1 - (q & 1)))[0]
    fef[0] = fe.astype(BF)
    fef[1] = ff.astype(BF)
    fef[2] = (fe * jnp.where((l & 95) == 0, 1.0 / D, 2.0 / D)).T.astype(BF)
    fef[3] = (ff * (2.0 / D)).T.astype(BF)
    ko = 4 * m + 1 + 2 * (q & 1) + 128 - 128 * (q >> 1)
    c, s_ = ex(4 * ko)
    sg = (1 - 2 * (q & 1)).astype(F32)
    for (i, j), v in {(0, 0): c, (0, 1): s_, (1, 0): s_ * sg, (1, 1): -c * sg}.items():
        foo[0, 128 * i:128 * i + 128, 128 * j:128 * j + 128] = v.astype(BF)
        foo[1, 128 * j:128 * j + 128, 128 * i:128 * i + 128] = (v * (2.0 / D)).T.astype(BF)
    n1, im = ((l >> 4) << 3) | (l & 7), (l >> 3) & 1
    a, b = ex(32 * n1, -Q * im, 8)
    a, b = jnp.concatenate([a, b], 0), jnp.concatenate([b, -a], 0)
    tc, ts = ex(n1, 0, 4)
    tw[2, 0:32, :] = tc
    tw[2, 32:64, :] = ts
    tw[3], tw[4] = a[:64], b[:64]

    def mk(k2):
        a, b = jnp.concatenate([tw[3], tw[4]], 0), jnp.concatenate([tw[4], -tw[3]], 0)
        v = a * tw[2, pl.ds(k2, 1), :] - b * tw[2, pl.ds(k2 + 32, 1), :]
        fs[k2] = v.astype(BF)
        gs[k2] = (v * (1.0 / S)).T.astype(BF)
    v = jnp.concatenate(ex(32 * (l & 63), -Q * (l >> 6), 8), 0)
    f64[0] = v.astype(BF)
    f64[1] = v.T.astype(BF)
    ok = ((l < 32) & ((r >> 4) == (l & 1)))[:32]
    cc, tt = ex(64 * l, 0, 2), ex(l, 0, 8)
    c1[...] = jnp.zeros((128, 256), BF)
    for i in range(2):
        v = jnp.where(ok, jnp.concatenate([cc[i], cc[i]], 0), 0.0)
        c1[0:32, 128 * i:128 * i + 128] = v.astype(BF)
        tw[i] = tt[i]
    return mk


def _cmul_const(z, ang):
    r, i = z
    ang %= 32
    if ang == 0:
        return r, i
    if ang == 8:
        return -i, r
    if ang == 16:
        return -r, -i
    if ang == 24:
        return i, -r
    c, s = float(np.cos(2 * np.pi * ang / 32)), float(np.sin(2 * np.pi * ang / 32))
    if ang % 8 == 4:
        if c * s > 0:
            return (r - i) * c, (r + i) * c
        return (r + i) * c, (i - r) * c
    return r * c - i * s, r * s + i * c


def _fft(z, sign):
    n = len(z)
    if n == 1:
        return z
    if n == 2:
        (ar, ai), (br, bi) = z
        return [(ar + br, ai + bi), (ar - br, ai - bi)]
    q = n // 4
    sub = [[], [], [], []]
    for m in range(q):
        (ar, ai), (br, bi), (cr, ci), (dr, di) = z[m], z[m + q], z[m + 2 * q], z[m + 3 * q]
        sr, si, tr, ti = ar + cr, ai + ci, ar - cr, ai - ci
        ur, ui, vr, vi = br + dr, bi + di, br - dr, bi - di
        o = [(sr + ur, si + ui), (tr + vi, ti - vr), (sr - ur, si - ui), (tr - vi, ti + vr)]
        if sign > 0:
            o[1], o[3] = o[3], o[1]
        for r in range(4):
            sub[r].append(_cmul_const(o[r], sign * r * m * (32 // n)))
    sub = [_fft(s_, sign) for s_ in sub]
    return [sub[k % 4][k // 4] for k in range(n)]


def _dot(a, b):
    return jnp.dot(a, b, preferred_element_type=F32)


def _body(x_h, wr_h, wi_h, w1_h, w2_h, gw, o_h, gidx, fef, foo, c1, f64, gt, tw, w1t,
          x, wr, wi, w1, w2, fs, gs, u, wt, wm, wn, vn, ob, sem, osem):
    R = 256
    xc = [pltpu.make_async_copy(x_h.at[pl.ds(c * R, R)], x.at[pl.ds(c * R, R)], sem.at[c])
          for c in range(8)]
    oth = [pltpu.make_async_copy(a, b_, sem.at[8 + n]) for n, (a, b_) in enumerate(
        [(w1_h, w1t), (w2_h, w2), (wr_h, wr), (wi_h, wi)])]
    for c in (0, 4, 1, 5, 2, 6, 3, 7):
        xc[c].start()
    oth[0].start()

    mk = _gen(gidx, fef, foo, fs, gs, c1, f64, tw)
    for c in oth[1:]:
        c.start()
    gwv = jnp.concatenate([gw[t:t + 1] for t in range(4)], 1)
    lane = jax.lax.broadcasted_iota(jnp.int32, (R, 128), 1)
    elane = (lane // 32) % 2 == 0
    lane64 = lane[:64]

    vn[...] = jnp.zeros((64, 128), F32)
    @pl.loop(0, 4)
    def _(c):
        for c_ in (c, c + 4):
            rr = pl.ds(pl.multiple_of(c_ * R, R), R)
            pltpu.make_async_copy(x_h.at[rr], x.at[rr], sem.at[c_]).wait()
        lo = x[pl.ds(pl.multiple_of(c * R, R), R), :].astype(F32)
        hi = x[pl.ds(pl.multiple_of(1024 + c * R, R), R), :].astype(F32)
        for p in range(2):
            v = lo + hi if p == 0 else lo - hi
            x0, x1, x2, x3 = (v[:, 128 * t:128 * t + 128] for t in range(4))
            a, b = x0 + x2, x1 + x3
            e = _dot((a + b).astype(BF), fef[0])
            f = _dot((a - b).astype(BF), fef[1])
            z = _dot(jnp.concatenate([x0 - x2, x1 - x3], axis=1).astype(BF), foo[0])
            rows = pl.ds(pl.multiple_of(p * 1024 + c * R, R), R)
            u[rows, 0:128] = jnp.where(elane, e, f)
            u[rows, 128:256] = jnp.where(lane == 0, 0.0, pltpu.roll(jnp.where(elane, f, e), 96, 1))
            u[rows, 256:512] = z
            acc = vn[...]
            for t in range(4):
                j = p * 16 + c * 4 + t
                acc = jnp.where(lane64 == j, pltpu.roll(e[64 * t:64 * t + 64], j + 96, 1), acc)
            vn[...] = acc

    def ffn(r0, hs, i):
        if i < 4:
            h = _dot(x[pl.ds(r0, R), :], w1[:, 384 * i:min(384 * i + 384, F)]) * 0.5
            hs.append((h * jnp.tanh(h) + h).astype(BF))
            if i == 3:
                hs.append(jnp.concatenate(hs, 1))
        else:
            c = 128 * (i - 4)
            ob[pl.ds(r0, R), c:c + 128] = _dot(hs[-1], w2[:, c:c + 128])

    def prep_w(r0):
        for n, w in enumerate((wr, wi)):
            ta = pltpu.bitcast(w[0:128, pl.ds(r0, 512)].T, jnp.int32)
            tb = pltpu.bitcast(w[128:256, pl.ds(r0, 512)].T, jnp.int32)
            ia = jnp.broadcast_to(gidx[0][None], (32, 8, 128)).reshape(256, 128)
            ib = jnp.broadcast_to(gidx[1][None], (32, 8, 128)).reshape(256, 128)
            ta = jnp.take_along_axis(ta, ia, axis=1)
            tb = jnp.take_along_axis(tb, ib, axis=1)
            va = pltpu.bitcast(jnp.where(lane < 64, ta, tb), BF).astype(F32)
            vb = pltpu.bitcast(jnp.where(lane < 64, tb, ta), BF).astype(F32)
            for i in range(16):
                rr = pl.ds((r0 // 32 + i) * 33, 32)
                wm[n, rr, :] = va[32 * i:32 * i + 32]
                wm[2 + n, rr, :] = vb[32 * i:32 * i + 32]
            col = jnp.broadcast_to(w[256:257, pl.ds(r0, 512)].astype(F32), (128, 512)).T
            rr = jax.lax.broadcasted_iota(jnp.int32, (512, 128), 0)
            ll = jax.lax.broadcasted_iota(jnp.int32, (512, 128), 1)
            col = jnp.where(rr % 32 == ll, col, 0.0)
            wn[n, pl.ds(pl.multiple_of(r0 // 32, 16), 16), :] = col.reshape(16, 32, 128).sum(axis=1)

    oth[0].wait()
    w1[...] = w1t[...].T
    oth[1].wait()
    oth[2].wait()
    oth[3].wait()

    def p2(it, _):
        hs = []
        prep_w(pl.multiple_of(it * 512, 512))
        for gg in range(2):
            g = it * 2 + gg
            for p in range(2):
                for t in range(2):
                    ffn(pl.multiple_of(it * R, R), hs, gg * 4 + p * 2 + t)
                    mk(it * 8 + gg * 4 + p * 2 + t)
                    z = []
                    for m in range(16):
                        rows = pl.ds(pl.multiple_of(p * 1024 + m * 64 + g * 8, 8), 8)
                        z.append(_cmul_const((u[rows, 256 * t:256 * t + 128],
                                              u[rows, 256 * t + 128:256 * t + 256]), -m * p))
                    z = _fft(z, -1)
                    for q in range(16):
                        wt[p + 2 * q, pl.ds(pl.multiple_of(g * 16, 16), 16), 128 * t:128 * t + 128] = (
                            jnp.concatenate(z[q], axis=0).astype(BF))
        return 0

    jax.lax.fori_loop(0, 4, p2, 0)

    t_ = _dot(vn[...].astype(BF), c1[...])
    tr, ti = t_[:, :128], t_[:, 128:]
    y = _dot(f64[0], jnp.concatenate([tr * tw[0] - ti * tw[1], tr * tw[1] + ti * tw[0]], 0).astype(BF))
    yr, yi = y[:64], y[64:]
    y = _dot(f64[1], jnp.concatenate([yr * wn[0] - yi * wn[1], yr * wn[1] + yi * wn[0]], 0).astype(BF))
    tr, ti = y[:64], y[64:]
    vn[...] = (1.0 / S) * jax.lax.dot_general(jnp.concatenate([tr * tw[0] + ti * tw[1], ti * tw[0] - tr * tw[1]], 1).astype(BF), c1[...], (((1,), (1,)), ((), ())), preferred_element_type=F32)

    @pl.loop(0, 32, unroll=8)
    def _(k2):
        y = _dot(fs[k2], wt[k2])
        o = []
        for t in range(2):
            yr, yi = y[:64, 128 * t:128 * t + 128], y[64:, 128 * t:128 * t + 128]
            ar = wm[2 * t, pl.ds(k2, 64, stride=33), :]
            ai = wm[2 * t + 1, pl.ds(k2, 64, stride=33), :]
            o.append(jnp.concatenate([yr * ar - yi * ai, yr * ai + yi * ar], 0).astype(BF))
        zz = _dot(gs[k2], jnp.concatenate(o, 1))
        zr_ = jnp.concatenate([zz[16 * i:16 * i + 8] for i in range(8)], 0)
        zi_ = jnp.concatenate([zz[16 * i + 8:16 * i + 16] for i in range(8)], 0)
        rows = pl.ds(pl.multiple_of((k2 % 2) * 1024 + (k2 // 2) * 64, 64), 64)
        for t in range(2):
            u[rows, 256 * t:256 * t + 128] = zr_[:, 128 * t:128 * t + 128]
            u[rows, 256 * t + 128:256 * t + 256] = zi_[:, 128 * t:128 * t + 128]

    def p4(it, _):
        hs = []
        for gg in range(2):
            g = it * 2 + gg
            for p in range(2):
                for t in range(2):
                    ffn(pl.multiple_of(1024 + it * R, R), hs, gg * 4 + p * 2 + t)
                    gr = pl.ds(pl.multiple_of(it * 512 + (gg * 4 + p * 2 + t) * 64, 64), 64)
                    s = jnp.sum((x[gr, :] * gwv).astype(F32), axis=1, keepdims=True)
                    gt[gr, :] = jax.nn.sigmoid(jnp.broadcast_to(s, (64, 128)))
                    rows = [pl.ds(pl.multiple_of(p * 1024 + m * 64 + g * 8, 8), 8) for m in range(16)]
                    z = _fft([(u[r, 256 * t:256 * t + 128], u[r, 256 * t + 128:256 * t + 256])
                              for r in rows], 1)
                    for m in range(16):
                        zr, zi = _cmul_const(z[m], m * p)
                        u[rows[m], 256 * t:256 * t + 128] = zr
                        u[rows[m], 256 * t + 128:256 * t + 256] = zi
        return 0

    jax.lax.fori_loop(0, 4, p4, 0)

    @pl.loop(0, 4)
    def _(c):
        ys = []
        for p in range(2):
            rows = pl.ds(pl.multiple_of(p * 1024 + c * R, R), R)
            re = u[rows, 0:128]
            im = pltpu.roll(u[rows, 128:256], 32, 1)
            vv = vn[...]
            ny = jnp.concatenate([pltpu.roll(vv, 32 - (p * 16 + c * 4 + t), 1) for t in range(4)], 0)
            e = _dot(jnp.where(lane == 32, ny, jnp.where(elane, re, im)).astype(BF), fef[2])
            f = _dot(jnp.where(elane, im, re).astype(BF), fef[3])
            z = _dot(u[rows, 256:512].astype(BF), foo[1])
            a, b = e + f, e - f
            cc, dd = z[:, :128], z[:, 128:]
            ys.append(jnp.concatenate([a + cc, b + dd, a - cc, b - dd], 1))
        for hh in range(2):
            rows = pl.ds(pl.multiple_of(hh * 1024 + c * R, R), R)
            a = ys[0] + ys[1] if hh == 0 else ys[0] - ys[1]
            g = jnp.concatenate([gt[rows, :]] * 4, 1)
            x[rows, :] = (g * a + (1.0 - g) * ob[rows, :]).astype(BF)
            cp = pltpu.make_async_copy(x.at[rows], o_h.at[rows], osem.at[c * 2 + hh])
            cp.start()
    for i in range(8):
        rr = pl.ds((i % 2) * 1024 + (i // 2) * R, R)
        pltpu.make_async_copy(x.at[rr], o_h.at[rr], osem.at[i]).wait()


@jax.jit
def pallas_gated_mix__spectral_gfnet__dense_activation_silu__prompt_kernel(
        A_x, A_w_r, A_w_i, B_x, B_w1, B_w2, gate_w):
    hbm = pl.BlockSpec(memory_space=pltpu.HBM)
    vm = pl.BlockSpec(memory_space=pltpu.VMEM)
    V = pltpu.VMEM
    out = pl.pallas_call(
        _body,
        out_shape=jax.ShapeDtypeStruct((S, D), BF),
        in_specs=[hbm] * 5 + [vm],
        out_specs=hbm,
        scratch_shapes=[V((2, 8, 128), jnp.int32), V((4, 128, 128), BF), V((2, 256, 256), BF), V((128, 256), BF),
                        V((2, 128, 128), BF), V((S, 128), F32), V((5, 64, 128), F32), V((F, D), BF),
                        V((S, D), BF), V((257, S), BF), V((257, S), BF), V((D, F), BF), V((F, D), BF),
                        V((32, 128, 128), BF), V((32, 128, 128), BF), V((S, D), F32),
                        V((32, 128, 256), BF), V((4, 64 * 33, 128), F32), V((2, 64, 128), F32),
                        V((64, 128), F32), V((S, D), F32),
                        pltpu.SemaphoreType.DMA((14,)), pltpu.SemaphoreType.DMA((8,))],
        compiler_params=pltpu.CompilerParams(vmem_limit_bytes=100 * 1024 * 1024),
    )(A_x.reshape(S, D), A_w_r.T, A_w_i.T, B_w1.T, B_w2, gate_w.reshape(4, 128))
    return out.reshape(1, S, D)
```
